```python
import os as _os
_os.environ.setdefault('JAX_PLATFORMS', 'cpu')
import jax
import jax.numpy as jnp

def _softmax(x, axis=-1):
    return jax.nn.softmax(x, axis=axis)

def _gelu(x):
    return jax.nn.gelu(x, approximate=True)

def _silu(x):
    return jax.nn.silu(x)

def _sigmoid(x):
    return jax.nn.sigmoid(x)

def _layernorm(x, axis=-1, eps=1e-05):
    m = jnp.mean(x, axis=axis, keepdims=True)
    v = jnp.var(x, axis=axis, keepdims=True)
    return (x - m) / jnp.sqrt(v + eps)

def _scatter_add(tgt, idx, src, axis=0):
    return tgt.at[idx].add(src)

def _segment_sum(src, seg, n):
    return jax.ops.segment_sum(src, seg, n)

class _Rng:

    def __init__(self, key):
        self._k = key

    def _next(self):
        self._k, sub = jax.random.split(self._k)
        return sub

    def normal(self, shape):
        return jax.random.normal(self._next(), shape, dtype=jnp.bfloat16)

    def randint(self, lo, hi, shape):
        return jax.random.randint(self._next(), shape, lo, hi, dtype=jnp.int32)

    def uniform(self, shape, lo=0.0, hi=1.0):
        return jax.random.uniform(self._next(), shape, jnp.bfloat16, lo, hi)

    def permutation(self, n):
        return jax.random.permutation(self._next(), n)
kernel_name = 'standalone__autoregressive_conv_wavenet__speech'

def setup_inputs():
    _rng = _Rng(jax.random.key(int.from_bytes(__import__("os").urandom(4), "little")))
    _w = lambda a: (lambda t: t.astype(jnp.bfloat16) if jnp.issubdtype(t.dtype, jnp.floating) else t)(jnp.asarray(a))
    B, T, D, K = (2, 4000, 512, 31)
    return {'x': _w((lambda *s: _rng.normal(s) * 0.05)(B, T, D)), 'w': _w((lambda *s: _rng.normal(s) * 0.05)(K, D, 2 * D)), 'w_o': _w((lambda *s: _rng.normal(s) * 0.05)(D, D))}

def reference(x, w, w_o):
    B, T, D = x.shape
    K = w.shape[0]
    dil = 2
    pad = (K - 1) * dil
    xp = jnp.pad(x, ((0, 0), (pad, 0), (0, 0)))
    h = jnp.einsum('btc,cd->btd', xp[:, pad:pad + T, :], w[0])
    for i in range(1, K):
        off = pad - i * dil
        h = h + jnp.einsum('btc,cd->btd', xp[:, off:off + T, :], w[i])
    f = h[..., :D].copy()
    g = h[..., D:].copy()
    z = jnp.tanh(f) * _sigmoid(g)
    return z @ w_o
```

```python
import functools

import jax
import jax.numpy as jnp
import jax.experimental.pallas as pl
import jax.experimental.pallas.tpu as pltpu

_DIL = 2
_SUB = 8


def _kernel(x_ref, w_ref, wo_ref, o_ref, win_ref, cp_ref, *, tm, n_taps, d):
    j = pl.program_id(1)
    qmax = (n_taps - 1) // _SUB
    halo = 16 * (qmax + 1)
    t0 = pl.multiple_of(j * tm, 16)

    win_ref[pl.ds(halo, tm), :] = x_ref[pl.ds(t0, tm), :]
    hstart = pl.multiple_of(jnp.maximum(t0 - halo, 0), 16)
    hrows = x_ref[pl.ds(hstart, halo), :]
    win_ref[pl.ds(0, halo), :] = jnp.where(j > 0, hrows, jnp.zeros_like(hrows))

    ncp = tm + 16 * qmax
    for r in range(_SUB):
        cp_ref[r] = win_ref[pl.ds(16 - _DIL * r, ncp), :]

    lhs = jnp.concatenate(
        [cp_ref[i % _SUB, pl.ds(16 * (qmax - i // _SUB), tm), :] for i in range(n_taps)], axis=1)
    h = jnp.dot(lhs, w_ref[...], preferred_element_type=jnp.float32)

    z = jnp.tanh(h[:, :d]) * jax.nn.sigmoid(h[:, d:])
    o_ref[...] = jnp.dot(z.astype(jnp.bfloat16), wo_ref[...],
                         preferred_element_type=jnp.float32).astype(o_ref.dtype)


@jax.jit
def pallas_standalone__autoregressive_conv_wavenet__speech_kernel(
    x: jax.Array,
    w: jax.Array,
    w_o: jax.Array,
):
    b, t, d = x.shape
    n_taps = w.shape[0]
    tm = 800
    assert t % tm == 0 and tm % 16 == 0
    qmax = (n_taps - 1) // _SUB
    halo = 16 * (qmax + 1)
    assert halo >= (n_taps - 1) * _DIL
    w2 = w.reshape(n_taps * d, 2 * d)

    kernel = functools.partial(_kernel, tm=tm, n_taps=n_taps, d=d)
    return pl.pallas_call(
        kernel,
        grid=(b, t // tm),
        in_specs=[
            pl.BlockSpec((None, t, d), lambda bi, j: (bi, 0, 0)),
            pl.BlockSpec((n_taps * d, 2 * d), lambda bi, j: (0, 0), pipeline_mode=pl.Buffered(1)),
            pl.BlockSpec((d, d), lambda bi, j: (0, 0)),
        ],
        out_specs=pl.BlockSpec((None, tm, d), lambda bi, j: (bi, j, 0)),
        out_shape=jax.ShapeDtypeStruct((b, t, d), x.dtype),
        scratch_shapes=[
            pltpu.VMEM((tm + halo, d), jnp.bfloat16),
            pltpu.VMEM((_SUB, tm + 16 * qmax, d), jnp.bfloat16),
        ],
        compiler_params=pltpu.CompilerParams(
            dimension_semantics=("arbitrary", "arbitrary"),
            vmem_limit_bytes=110 * 1024 * 1024,
        ),
    )(x, w2, w_o)
```

```python
import functools

import jax
import jax.numpy as jnp
import jax.experimental.pallas as pl
import jax.experimental.pallas.tpu as pltpu

_DIL = 2
_SUB = 8
_LANE = 128


def _kernel(xc_ref, xn_ref, w_hbm, wo_ref, o_ref, win_ref, cp_ref, z_ref, wv_ref, sem,
            *, tm, n_taps, d, nt):
    b = pl.program_id(0)
    j = pl.program_id(1)
    qmax = (n_taps - 1) // _SUB
    halo = 16 * (qmax + 1)
    ncp = tm + 16 * qmax
    nc = d // _LANE
    first = jnp.logical_and(b == 0, j == 0)
    cur = (b * nt + j) % 2
    nxt = 1 - cur

    def w_copy(t):
        col = pl.multiple_of(t * _LANE, _LANE)
        return pltpu.make_async_copy(w_hbm.at[:, pl.ds(col, _LANE)],
                                     wv_ref.at[:, pl.ds(col, _LANE)], sem.at[t])

    @pl.when(first)
    def _():
        for c in range(nc):
            w_copy(c).start()
            w_copy(c + nc).start()
        win_ref[pl.ds(0, halo), :] = jnp.zeros((halo, d), win_ref.dtype)
        win_ref[pl.ds(halo, tm), :] = xc_ref[...]
        for r in range(_SUB):
            cp_ref[cur, r] = win_ref[pl.ds(16 - _DIL * r, ncp), :]

    nrows = ncp - halo
    ch = 16 * (-(-(nrows // 16) // nc))

    def col_group(c, carry):
        @pl.when(first)
        def _():
            w_copy(c).wait()

        cf = pl.multiple_of(c * _LANE, _LANE)
        cg = pl.multiple_of(d + c * _LANE, _LANE)
        lhs = jnp.concatenate(
            [cp_ref[cur, i % _SUB, pl.ds(16 * (qmax - i // _SUB), tm), :] for i in range(n_taps)],
            axis=1)
        f = jnp.dot(lhs, wv_ref[:, pl.ds(cf, _LANE)], preferred_element_type=jnp.float32)

        @pl.when(first)
        def _():
            w_copy(c + nc).wait()

        g = jnp.dot(lhs, wv_ref[:, pl.ds(cg, _LANE)], preferred_element_type=jnp.float32)
        z_ref[:, pl.ds(cf, _LANE)] = (jnp.tanh(f) * jax.nn.sigmoid(g)).astype(z_ref.dtype)

        u0 = pl.multiple_of(halo + jnp.minimum(c * ch, nrows - ch), 16)
        slab = xn_ref[pl.ds(pl.multiple_of(u0 - halo, 16), ch + 16), :]
        for r in range(_SUB):
            cp_ref[nxt, r, pl.ds(u0, ch), :] = slab[16 - _DIL * r: 16 - _DIL * r + ch, :]
        return carry

    jax.lax.fori_loop(0, nc, col_group, 0)

    tail = xc_ref[pl.ds(tm - halo, halo), :]
    tail = jnp.where(j == nt - 1, jnp.zeros_like(tail), tail)
    hist = jnp.concatenate([tail, xn_ref[pl.ds(0, 16), :]], axis=0)
    for r in range(_SUB):
        cp_ref[nxt, r, pl.ds(0, halo), :] = hist[16 - _DIL * r: 16 - _DIL * r + halo, :]

    o_ref[...] = jnp.dot(z_ref[...], wo_ref[...],
                         preferred_element_type=jnp.float32).astype(o_ref.dtype)


@jax.jit
def pallas_standalone__autoregressive_conv_wavenet__speech_kernel(
    x: jax.Array,
    w: jax.Array,
    w_o: jax.Array,
):
    b, t, d = x.shape
    n_taps = w.shape[0]
    tm = 800
    assert t % tm == 0 and tm % 16 == 0
    nt = t // tm
    qmax = (n_taps - 1) // _SUB
    halo = 16 * (qmax + 1)
    assert halo >= (n_taps - 1) * _DIL and tm >= halo
    w2 = w.reshape(n_taps * d, 2 * d)

    def next_tile(bi, j):
        last = j == nt - 1
        return (jnp.where(last, jnp.minimum(bi + 1, b - 1), bi), jnp.where(last, 0, j + 1), 0)

    kernel = functools.partial(_kernel, tm=tm, n_taps=n_taps, d=d, nt=nt)
    return pl.pallas_call(
        kernel,
        grid=(b, nt),
        in_specs=[
            pl.BlockSpec((None, tm, d), lambda bi, j: (bi, j, 0)),
            pl.BlockSpec((None, tm, d), next_tile),
            pl.BlockSpec(memory_space=pl.ANY),
            pl.BlockSpec((d, d), lambda bi, j: (0, 0)),
        ],
        out_specs=pl.BlockSpec((None, tm, d), lambda bi, j: (bi, j, 0)),
        out_shape=jax.ShapeDtypeStruct((b, t, d), x.dtype),
        scratch_shapes=[
            pltpu.VMEM((tm + halo, d), jnp.bfloat16),
            pltpu.VMEM((2, _SUB, tm + 16 * qmax, d), jnp.bfloat16),
            pltpu.VMEM((tm, d), jnp.bfloat16),
            pltpu.VMEM((n_taps * d, 2 * d), jnp.bfloat16),
            pltpu.SemaphoreType.DMA((2 * d // _LANE,)),
        ],
        compiler_params=pltpu.CompilerParams(
            dimension_semantics=("arbitrary", "arbitrary"),
            vmem_limit_bytes=110 * 1024 * 1024,
        ),
    )(x, x, w2, w_o)
```

```python
import functools

import jax
import jax.numpy as jnp
import jax.experimental.pallas as pl
import jax.experimental.pallas.tpu as pltpu

_DIL = 2
_SUB = 8
_NCP = 4
_LANE = 128


def _kernel(x_hbm, w_hbm, wo_hbm, o_ref,
            xb_ref, win_ref, cp_ref, tail_ref, act_ref, z_ref, wv_ref, wo_ref, sem,
            *, nb, tm, n_taps, d, nt):
    j = pl.program_id(0)
    qmax = (n_taps - 1) // _SUB
    halo = 16 * (qmax + 2)
    ncp = tm + halo - 16
    nc = d // _LANE
    first = j == 0
    cur = j % 2
    nxt = 1 - cur

    def w_copy(t):
        col = pl.multiple_of(t * _LANE, _LANE)
        return pltpu.make_async_copy(w_hbm.at[:, pl.ds(col, _LANE)],
                                     wv_ref.at[:, pl.ds(col, _LANE)], sem.at[t])

    def wo_copy():
        return pltpu.make_async_copy(wo_hbm, wo_ref, sem.at[2 * nc])

    def x_first_copy():
        return pltpu.make_async_copy(x_hbm.at[:, pl.ds(0, tm), :],
                                     win_ref.at[:, pl.ds(halo, tm), :], sem.at[2 * nc + 1])

    def x_copy(tile, slot):
        rows = pl.ds(pl.multiple_of(tile * tm, 16), tm)
        return pltpu.make_async_copy(x_hbm.at[:, rows, :], xb_ref.at[slot], sem.at[2 * nc + 2 + slot])

    @pl.when(first)
    def _():
        x_first_copy().start()
        w_copy(0).start()
        if nt > 1:
            x_copy(1, 1).start()
        w_copy(nc).start()
        for c in range(1, nc):
            w_copy(c).start()
            w_copy(c + nc).start()
        wo_copy().start()
        if nt > 2:
            x_copy(2, 0).start()
        act_ref[...] = jnp.zeros_like(act_ref)
        for bi in range(nb):
            win_ref[bi, pl.ds(0, halo), :] = jnp.zeros((halo, d), win_ref.dtype)
        x_first_copy().wait()
        for bi in range(nb):
            tail_ref[bi] = win_ref[bi, pl.ds(tm, halo), :]
            for r in range(_NCP):
                cp_ref[cur, r, bi] = win_ref[bi, pl.ds(16 - _DIL * r, ncp), :]

    nslot = (j + 1) % 2

    @pl.when(j + 1 < nt)
    def _():
        x_copy(j + 1, nslot).wait()

    @pl.when(jnp.logical_and(j >= 1, j + 2 < nt))
    def _():
        x_copy(j + 2, j % 2).start()

    nrows = ncp - halo
    ch = 16 * (-(-(nrows // 16) // (2 * nc)))

    def col_tile(i, carry):
        is_g = (i % 2) == 1
        cgrp = i // 2
        t = (i % 2) * nc + cgrp

        @pl.when(first)
        def _():
            w_copy(t).wait()

        lhs = jnp.concatenate(
            [jnp.concatenate(
                [cp_ref[cur, k % _NCP, bi,
                        pl.ds(halo - 16 - 16 * (k // _SUB) - 8 * ((k % _SUB) // _NCP), tm), :]
                 for bi in range(nb)], axis=0)
             for k in range(n_taps)], axis=1)
        col = pl.multiple_of(t * _LANE, _LANE)
        a = jnp.dot(lhs, wv_ref[:, pl.ds(col, _LANE)], preferred_element_type=jnp.float32)

        half = jnp.where(is_g, 0.5, 1.0).astype(jnp.float32)
        act = jnp.tanh(a * half) * half + jnp.where(is_g, 0.5, 0.0).astype(jnp.float32)
        zc = pl.multiple_of(cgrp * _LANE, _LANE)
        z_ref[:, pl.ds(zc, _LANE)] = jnp.where(is_g, act_ref[...] * act, act).astype(z_ref.dtype)
        act_ref[...] = act

        u0 = pl.multiple_of(halo + jnp.minimum(i * ch, nrows - ch), 16)
        for bi in range(nb):
            slab = xb_ref[nslot, bi, pl.ds(pl.multiple_of(u0 - halo, 16), ch + 16), :]
            for r in range(_NCP):
                cp_ref[nxt, r, bi, pl.ds(u0, ch), :] = slab[16 - _DIL * r: 16 - _DIL * r + ch, :]
        return carry

    jax.lax.fori_loop(0, 2 * nc, col_tile, 0)

    @pl.when(first)
    def _():
        wo_copy().wait()

    for bi in range(nb):
        hist = jnp.concatenate([tail_ref[bi], xb_ref[nslot, bi, pl.ds(0, 16), :]], axis=0)
        for r in range(_NCP):
            cp_ref[nxt, r, bi, pl.ds(0, halo), :] = hist[16 - _DIL * r: 16 - _DIL * r + halo, :]
        tail_ref[bi] = xb_ref[nslot, bi, pl.ds(tm - halo, halo), :]

    out = jnp.dot(z_ref[...], wo_ref[...], preferred_element_type=jnp.float32)
    o_ref[...] = out.reshape(nb, tm, d).astype(o_ref.dtype)


@jax.jit
def pallas_standalone__autoregressive_conv_wavenet__speech_kernel(
    x: jax.Array,
    w: jax.Array,
    w_o: jax.Array,
):
    b, t, d = x.shape
    n_taps = w.shape[0]
    tm = 800
    assert t % tm == 0 and tm % 16 == 0
    nt = t // tm
    qmax = (n_taps - 1) // _SUB
    halo = 16 * (qmax + 2)
    assert halo - 16 >= (n_taps - 1) * _DIL and tm >= halo
    w2 = w.reshape(n_taps * d, 2 * d)

    kernel = functools.partial(_kernel, nb=b, tm=tm, n_taps=n_taps, d=d, nt=nt)
    return pl.pallas_call(
        kernel,
        grid=(nt,),
        in_specs=[
            pl.BlockSpec(memory_space=pl.ANY),
            pl.BlockSpec(memory_space=pl.ANY),
            pl.BlockSpec(memory_space=pl.ANY),
        ],
        out_specs=pl.BlockSpec((b, tm, d), lambda j: (0, j, 0)),
        out_shape=jax.ShapeDtypeStruct((b, t, d), x.dtype),
        scratch_shapes=[
            pltpu.VMEM((2, b, tm, d), jnp.bfloat16),
            pltpu.VMEM((b, tm + halo, d), jnp.bfloat16),
            pltpu.VMEM((2, _NCP, b, tm + halo - 16, d), jnp.bfloat16),
            pltpu.VMEM((b, halo, d), jnp.bfloat16),
            pltpu.VMEM((b * tm, _LANE), jnp.float32),
            pltpu.VMEM((b * tm, d), jnp.bfloat16),
            pltpu.VMEM((n_taps * d, 2 * d), jnp.bfloat16),
            pltpu.VMEM((d, d), jnp.bfloat16),
            pltpu.SemaphoreType.DMA((2 * d // _LANE + 4,)),
        ],
        compiler_params=pltpu.CompilerParams(
            dimension_semantics=("arbitrary",),
            vmem_limit_bytes=110 * 1024 * 1024,
        ),
    )(x, w2, w_o)
```
